```python
import os as _os
_os.environ.setdefault("JAX_PLATFORMS", "cpu")
import jax
import jax.numpy as jnp

def _softmax(x, axis=-1):
    return jax.nn.softmax(x, axis=axis)
def _gelu(x):
    return jax.nn.gelu(x, approximate=True)
def _silu(x):
    return jax.nn.silu(x)
def _sigmoid(x):
    return jax.nn.sigmoid(x)
def _layernorm(x, axis=-1, eps=1e-5):
    m = jnp.mean(x, axis=axis, keepdims=True)
    v = jnp.var(x, axis=axis, keepdims=True)
    return (x - m) / jnp.sqrt(v + eps)
def _scatter_add(tgt, idx, src, axis=0):
    return tgt.at[idx].add(src)
def _segment_sum(src, seg, n):
    return jax.ops.segment_sum(src, seg, n)
class _Rng:
    def __init__(self, key):
        self._k = key
    def _next(self):
        self._k, sub = jax.random.split(self._k)
        return sub
    def normal(self, shape):
        return jax.random.normal(self._next(), shape, dtype=jnp.bfloat16)
    def randint(self, lo, hi, shape):
        return jax.random.randint(self._next(), shape, lo, hi, dtype=jnp.int32)
    def uniform(self, shape, lo=0.0, hi=1.0):
        return jax.random.uniform(self._next(), shape, jnp.bfloat16, lo, hi)
    def permutation(self, n):
        return jax.random.permutation(self._next(), n)


kernel_name = 'standalone__moe_arch_mod__prompt'

def setup_inputs():
    _rng = _Rng(jax.random.key(int.from_bytes(__import__("os").urandom(4), "little")))
    _w = (lambda a: (lambda t: t.astype(jnp.bfloat16) if jnp.issubdtype(t.dtype, jnp.floating) else t)(jnp.asarray(a)))
    B, S, D, F, C = 1, 2048, 576, 4608, 8
    return {
        "x": _w((lambda *s: _rng.normal(s) * 0.1)(B, S, D)),
        "w_r": _w((lambda *s: _rng.normal(s) * 0.1)(D)),
        "w_gate": _w((lambda *s: _rng.normal(s) * 0.1)(D, F)),
        "w_up": _w((lambda *s: _rng.normal(s) * 0.1)(D, F)),
        "w_down": _w((lambda *s: _rng.normal(s) * 0.1)(F, D)),
    }

def reference(x, w_r, w_gate, w_up, w_down):
    B, S, D = x.shape
    C = 8
    r = x @ w_r
    idx = jnp.argsort(-r, axis=-1)[:, :C]
    idx_e = jnp.repeat(idx.reshape(B, C, 1), D, axis=2)
    x_sel = jnp.take_along_axis(x, idx_e, axis=1)
    g = _silu(x_sel @ w_gate)
    u = x_sel @ w_up
    y = (g * u) @ w_down
    r_sel = _sigmoid(jnp.take_along_axis(r, idx, axis=1))
    y = y * r_sel.reshape(B, C, 1)
    b_off = (jnp.arange(B) * S).reshape(B, 1)
    flat_idx = (idx + b_off).reshape(B * C)
    zero = (x * 0.0).reshape(B * S, D)
    upd = _scatter_add(zero, flat_idx, y.reshape(B * C, D), axis=0)
    return x + upd.reshape(B, S, D)
```

```python
import functools
import jax
import jax.numpy as jnp
from jax import lax
from jax.experimental import pallas as pl
from jax.experimental.pallas import tpu as pltpu

bf16, f32, i32 = jnp.bfloat16, jnp.float32, jnp.int32
C = 8
LANES = 128
PERM = (0, 8, 4, 12, 2, 10, 6, 14, 1, 9, 5, 13, 3, 11, 7, 15)
NT = (((1,), (1,)), ((), ()))


def make(name="moe", R0=320, R=128, W=9, trig=8, ltail=8, lrows=(128, 128, 64), kchunks=(12, 12, 7, 5), perm=PERM,
         rm=4, rgap=3, tgap=1, gath=2, gathgap=3, resgap=1, gm=4, ggap=4, um=4, ugap=3, dm=4, dgap=3, lm=18, lgap=4,
         wprio=(0, 1), compute=True, lag=2, xlag=None, glag=None, ulag=None, quiet=0, semcheck=False, scopes=False, wplan=None, verbose=False):
    def kernel(x_hbm, wr_hbm, wg_hbm, wu_hbm, wd_hbm, o_hbm,
               xb, wrb, gb, ub, db, ob, g_sc, h_sc, col_sc, order, sems):
        D, S = xb.shape
        F = gb.shape[1]
        NB = S // LANES
        NF = F // LANES
        nh = (D - R0) // R
        assert sum(kchunks) == NF and R0 + nh * R == D and sum(lrows) == R0
        nk = len(kchunks)
        kstart = [sum(kchunks[:c]) for c in range(nk + 1)]
        nl = len(lrows)
        lstart = [sum(lrows[:c]) for c in range(nl + 1)]

        sem_count = [0]

        def new_sem():
            sem_count[0] += 1
            return sems.at[sem_count[0] - 1]

        def cp(src, dst, r0, rows, c0, cols, sem):
            return pltpu.make_async_copy(src.at[pl.ds(r0, rows), pl.ds(c0, cols)],
                                         dst.at[pl.ds(r0, rows), pl.ds(c0, cols)], sem)

        sem_z = new_sem()
        L = dict(x=[cp(x_hbm, xb, 0, R0, 0, S, new_sem())],
                 g=[cp(wg_hbm, gb, 0, R0, 0, F, new_sem())],
                 u=[cp(wu_hbm, ub, 0, R0, 0, F, new_sem())])
        for c in range(nl - 1):
            L[f"d{c}"] = [cp(wd_hbm, db, lstart[c], lrows[c], 0, F, new_sem())]
        L_last = [cp(wd_hbm, db, lstart[nl - 1], lrows[-1] - ltail, 0, F, sem_z)]
        L_tail = [cp(wd_hbm, db, R0 - ltail, ltail, 0, F, sem_z)] if ltail else []

        spec = []
        ends = {}
        for key, src, dst, j0, j1 in ([("x", x_hbm, xb, 0, NB), ("g", wg_hbm, gb, 0, NF), ("u", wu_hbm, ub, 0, NF)]
                                      + [(f"k{c}", wd_hbm, db, kstart[c], kstart[c + 1]) for c in range(nk)]):
            sem = new_sem()
            for j in range(j0, j1):
                for t in range(nh):
                    spec.append((src, dst, R0 + t * R, R, j * LANES, LANES, sem))
            ends[key] = len(spec)
        N = len(spec)
        issue, issued, w = [], W, W
        while issued < N:
            w_new = (wplan or {}).get(len(issue), w)
            k = min(max(0, 1 + w_new - (issued - len(issue))), N - issued)
            w = w_new
            issue.append(k)
            issued += k
        P = len(issue)
        assert trig <= N - P
        H = [cp(*s[:6], sem_z if i >= P else s[6]) for i, s in enumerate(spec)]
        wr_copy = pltpu.make_async_copy(wr_hbm, wrb, new_sem())
        sem_w = new_sem()

        tasks = [[] for _ in range(N)]
        late = []
        st = {}

        def at(i, fn):
            if i >= P - quiet:
                late.append(fn)
            else:
                tasks[i].append(fn)
            if verbose:
                print(i, getattr(fn, "func", fn).__name__, getattr(fn, "args", ()))

        sub = lax.broadcasted_iota(i32, (8, LANES), 0)
        lane = lax.broadcasted_iota(i32, (8, LANES), 1)

        def t_router_begin():
            wr_copy.wait()
            for c in L["x"]:
                c.wait()
            st["w8"] = jnp.broadcast_to(wrb[...].reshape(1, D), (8, D))
            st["r"] = [jnp.zeros((8, LANES), f32) for _ in range(NB // 8)]

        def t_router(j0, j1):
            res = jnp.dot(st["w8"], xb[:, j0 * LANES:j1 * LANES], preferred_element_type=f32)
            for j in range(j0, j1):
                part = res[:, (j - j0) * LANES:(j - j0 + 1) * LANES]
                st["r"][j // 8] = jnp.where(sub == j % 8, part, st["r"][j // 8])

        def t_keys():
            keys = []
            for q, r in enumerate(st["r"]):
                r = r.astype(bf16).astype(f32)
                bits = pltpu.bitcast(r, i32)
                bits = jnp.where(r == 0.0, 0, bits)
                mono = jnp.where(bits < 0, ~bits, bits | jnp.int32(-2 ** 31))
                u = lax.shift_right_logical(mono, 16)
                u = jnp.where(r != r, 0, u)
                idx = (q * 8 + sub) * LANES + lane
                keys.append(pltpu.bitcast((u << 11) | (S - 1 - idx) | 0x20000000, f32))
            st["keys"] = keys
            st["top"] = jnp.zeros((8, LANES), f32)

        def t_topk(c):
            m = functools.reduce(jnp.maximum, st["keys"])
            m = jnp.max(jnp.max(m, axis=0, keepdims=True), axis=1, keepdims=True)
            st["top"] = jnp.where(sub == c, m, st["top"])
            st["keys"] = [jnp.where(k == m, 0.0, k) for k in st["keys"]]

        def t_decode():
            bits = pltpu.bitcast(st["top"], i32)
            idx = (S - 1) - (bits & (S - 1))
            u = lax.shift_right_logical(bits, 11) & 0xFFFF
            rb = jnp.where(u >= 0x8000, u & 0x7FFF, u ^ 0xFFFF)
            r_sel = pltpu.bitcast(rb << 16, f32)
            st["gate"] = jax.nn.sigmoid(r_sel).astype(bf16).astype(f32)
            st["idx"] = idx
            tok = [idx[c, 0] for c in range(C)]
            st["tok"] = tok
            st["blk"] = [lax.shift_right_logical(t, 7) for t in tok]
            st["lane"] = [t & (LANES - 1) for t in tok]
            st["xs"] = jnp.zeros((8, D), f32)

        def t_order():
            hit = functools.reduce(jnp.bitwise_or, [jnp.int32(1) << b for b in st["blk"]])
            n1, n2 = jnp.int32(0), jnp.int32(NB - C)
            for j in perm:
                early = jnp.logical_and(((hit >> j) & 1) == 0, n1 < NB - C)
                order[jnp.where(early, n1, n2)] = jnp.int32(j)
                n1 = n1 + early.astype(i32)
                n2 = n2 + 1 - early.astype(i32)

        def t_gather(c0, c1):
            for c in range(c0, c1):
                col = pl.multiple_of(st["blk"][c] * LANES, LANES)
                words = pltpu.bitcast(xb[:, pl.ds(col, LANES)], i32)
                lanes = lax.broadcasted_iota(i32, words.shape, 1)
                only = pltpu.bitcast(jnp.where(lanes == st["lane"][c], words, 0), bf16)
                pick = jnp.ones((8, LANES), bf16)
                row = lax.dot_general(pick, only, NT, preferred_element_type=f32)
                rows = lax.broadcasted_iota(i32, (8, D), 0)
                st["xs"] = jnp.where(rows == c, row, st["xs"])

        def t_residual(j):
            v = xb[:, j * LANES:(j + 1) * LANES].astype(f32)
            ob[j] = (v + v * 0.0).astype(bf16)

        def t_wait(key):
            for c in L[key]:
                c.wait()

        def t_gate(j0, j1):
            g = jnp.dot(st["xs"].astype(bf16), gb[:, j0 * LANES:j1 * LANES], preferred_element_type=f32)
            g = g.astype(bf16).astype(f32)
            g_sc[:, j0 * LANES:j1 * LANES] = (g * jax.nn.sigmoid(g)).astype(bf16).astype(f32)

        def t_up(j0, j1):
            u = jnp.dot(st["xs"].astype(bf16), ub[:, j0 * LANES:j1 * LANES], preferred_element_type=f32)
            u = u.astype(bf16).astype(f32)
            h_sc[:, j0 * LANES:j1 * LANES] = g_sc[:, j0 * LANES:j1 * LANES] * u

        def t_down(key, r0, r1, j0, j1):
            h = h_sc[:, j0 * LANES:j1 * LANES].astype(bf16)
            y = lax.dot_general(h, db[r0:r1, j0 * LANES:j1 * LANES], NT, preferred_element_type=f32)
            st[key] = y if key not in st else st[key] + y

        if compute:
            i = ends["x"] - 1 + (lag if xlag is None else xlag)
            at(i, t_router_begin)
            for j in range(0, NB, rm):
                at(i, functools.partial(t_router, j, j + rm)); i += rgap
            at(i, t_keys)
            for c in range(C):
                at(i, functools.partial(t_topk, c)); i += tgap
            at(i, t_decode); i += 1
            at(i, t_order); i += 1
            for c in range(0, C, gath):
                at(i, functools.partial(t_gather, c, c + gath)); i += gathgap
            for j in range(NB):
                at(i, functools.partial(t_residual, j)); i += resgap
            i = max(i, ends["g"] - 1 + (lag if glag is None else glag))
            at(i, functools.partial(t_wait, "g"))
            for j in range(0, NF, gm):
                at(i, functools.partial(t_gate, j, min(j + gm, NF))); i += ggap
            i = max(i, ends["u"] - 1 + (lag if ulag is None else ulag))
            at(i, functools.partial(t_wait, "u"))
            for j in range(0, NF, um):
                at(i, functools.partial(t_up, j, min(j + um, NF))); i += ugap
            jobs = []
            for c in range(nk):
                if ends[f"k{c}"] <= P:
                    jobs.append((ends[f"k{c}"] - 1, "k", c))
            for c in range(nl - 1):
                jobs.append((ends["u"] + (N - ends["u"]) * lstart[c + 1] // R0 + lag, "l", c))
            done_k = set()
            for ready, kind, c in sorted(jobs):
                i = max(i, ready)
                if kind == "k":
                    done_k.add(c)
                    for j in range(kstart[c], kstart[c + 1], dm):
                        at(i, functools.partial(t_down, "yh", R0, D, j, min(j + dm, kstart[c + 1]))); i += dgap
                else:
                    at(i, functools.partial(t_wait, f"d{c}"))
                    for j in range(0, NF, lm):
                        at(i, functools.partial(t_down, f"yl{c}", lstart[c], lstart[c + 1], j, min(j + lm, NF))); i += lgap

        L["x"][0].start(priority=1)
        for i in range(W):
            H[i].start(priority=0)
        wr_copy.start(priority=0)
        for key, cs in L.items():
            if key != "x":
                for c in cs:
                    c.start(priority=1)
        for c in L_last + L_tail:
            c.start(priority=1)

        def run(fn, step=None):
            if scopes:
                with jax.named_scope(getattr(fn, "func", fn).__name__ + (f"_s{step}" if scopes == 2 else "")):
                    fn()
            else:
                fn()

        issued = W
        for i in range(P):
            H[i].wait()
            for c in H[issued:issued + issue[i]]:
                c.start(priority=0)
            issued += issue[i]
            for fn in tasks[i]:
                run(fn, i)
        if not compute:
            wr_copy.wait()
            for key, cs in L.items():
                for c in cs:
                    c.wait()
            for n in range(NB):
                order[n] = jnp.int32(perm[n])

        def out_copy(n):
            b = order[n]
            return pltpu.make_async_copy(ob.at[b], o_hbm.at[:, pl.ds(pl.multiple_of(b * LANES, LANES), LANES)], sem_w)

        writes = [out_copy(n) for n in range(NB)]

        def t_trigger():
            for c in L_last + H[P:N - trig]:
                c.wait()
            for n in range(NB - C):
                writes[n].start(priority=wprio[n % len(wprio)])

        def t_lastwait():
            for c in H[N - trig:] + L_tail:
                c.wait()

        def t_finish():
            for fn in late:
                fn()
            j0 = min(kstart[c] for c in range(nk) if c not in done_k)
            t_down("yh", R0, D, j0, NF)
            t_down(f"yl{nl - 1}", lstart[nl - 1], R0, 0, NF)
            y = jnp.concatenate([st[f"yl{c}"] for c in range(nl)] + [st["yh"]], axis=1)
            y = y.astype(bf16).astype(f32)
            y = (y * st["gate"][:, :1]).astype(bf16).astype(f32)
            xs = st["xs"]
            upd = (xs * 0.0 + y).astype(bf16).astype(f32)
            rows = xs + upd
            rows = jnp.concatenate([rows, jnp.zeros((LANES - 8, D), f32)], axis=0)
            col_sc[...] = pltpu.bitcast(rows.T.astype(bf16), i32)

        def t_patch(n):
            cols = col_sc[...]
            b = order[n]
            src = jnp.full((1, LANES), -1, i32)
            lane1 = lax.broadcasted_iota(i32, (1, LANES), 1)
            for c in range(C):
                src = jnp.where(lane1 + b * LANES == st["tok"][c], c, src)
            src = jnp.broadcast_to(src, cols.shape)
            new = jnp.take_along_axis(cols, jnp.maximum(src, 0), axis=1)
            new = pltpu.bitcast(new, bf16).astype(f32)
            keep = jnp.broadcast_to(src[:1] < 0, new.shape)
            ob[b] = jnp.where(keep, ob[b].astype(f32), new).astype(bf16)

        def t_drain():
            for c in writes:
                c.wait()

        run(t_trigger)
        run(t_lastwait)
        if compute:
            run(t_finish)
        def t_patches():
            nw = len(wprio)

            def body(k, _):
                for p in range(nw):
                    n = NB - C + k * nw + p
                    if compute:
                        t_patch(n)
                    out_copy(n).start(priority=wprio[p])
            lax.fori_loop(0, C // nw, body, None)
        run(t_patches)
        run(t_drain)

    def fn(x, w_r, w_gate, w_up, w_down):
        B, S, D = x.shape
        F = w_gate.shape[1]
        hbm = pl.BlockSpec(memory_space=pltpu.HBM)
        out = pl.pallas_call(
            kernel, name=name,
            out_shape=jax.ShapeDtypeStruct((D, S), x.dtype),
            in_specs=[hbm] * 5, out_specs=hbm,
            scratch_shapes=[
                pltpu.VMEM((D, S), bf16), pltpu.VMEM((D,), bf16),
                pltpu.VMEM((D, F), bf16), pltpu.VMEM((D, F), bf16), pltpu.VMEM((D, F), bf16),
                pltpu.VMEM((S // LANES, D, LANES), bf16),
                pltpu.VMEM((8, F), f32), pltpu.VMEM((8, F), f32),
                pltpu.VMEM((D // 2, LANES), i32),
                pltpu.SMEM((S // LANES,), i32),
                pltpu.SemaphoreType.DMA((9 + len(lrows) + len(kchunks),)),
            ],
            compiler_params=pltpu.CompilerParams(vmem_limit_bytes=64 * 1024 * 1024,
                                                 disable_semaphore_checks=not semcheck),
        )(x.reshape(S, D).T, w_r, w_gate, w_up, w_down.T)
        return out.T.reshape(B, S, D)

    return fn


@jax.jit
def pallas_standalone__moe_arch_mod__prompt_kernel(x, w_r, w_gate, w_up, w_down):
    return make("moe_mod", W=8, xlag=16, glag=10, ulag=4, quiet=4, R0=288, R=144, lrows=(128, 96, 64),
                kchunks=(12, 12, 6, 6), wprio=(0,), wplan={180: 9})(x, w_r, w_gate, w_up, w_down)
```

```python
import functools

import jax
import jax.numpy as jnp
from jax import lax
from jax.experimental import pallas as pl
from jax.experimental.pallas import tpu as pltpu

CAPACITY = 8
LANES = 128
PACED = 176
BAND = 32
OVERLAP = 8
LEAD = 2
TICK_ROWS = 17
TICK_DEPTH = 3
ROUTER_STEP, GATE_STEP, UP_STEP = 22, 61, 98
DOWN_TILES = (2,) * 13 + (6, 4)
BLOCK_ORDER = (0, 12, 8, 4, 1, 13, 9, 5, 2, 14, 10, 6, 3, 15, 11, 7)

bf16, f32, i32 = jnp.bfloat16, jnp.float32, jnp.int32
NT = (((1,), (1,)), ((), ()))


def _round(v):
    return v.astype(bf16).astype(f32)


def _tiles(j0, j1):
    return slice(j0 * LANES, j1 * LANES)


def _wait_all(buf, sem):
    pltpu.make_async_copy(buf, buf, sem).wait()


def _kernel(x_hbm, wr_hbm, wg_hbm, wu_hbm, wd_hbm, out_hbm,
            x_buf, wr_buf, wg_buf, wu_buf, wd_buf, out_buf,
            sel_ref, g_ref, h_ref, y_ref, routed_ref, order_ref,
            tick_src, tick_dst, sems, down_sems, tick_sems):
    D, S = x_buf.shape
    F = wg_buf.shape[1]
    n_blocks, n_tiles = S // LANES, F // LANES
    lo = D - PACED
    x_sem, wr_sem, wg_sem, wu_sem, mid_sem, overlap_sem, band_sem, out_sem = (sems.at[i] for i in range(8))
    down_edges = [sum(DOWN_TILES[:m]) for m in range(len(DOWN_TILES) + 1)]

    def rows_copy(src, dst, r0, r1, sem):
        return pltpu.make_async_copy(src.at[r0:r1], dst.at[r0:r1], sem)

    def tile_copies(src, dst, j, sem, top=0):
        cols = _tiles(j, j + 1)
        return [pltpu.make_async_copy(src.at[r:r + PACED, cols], dst.at[r:r + PACED, cols], sem)
                for r in (top, lo)]

    def wd_tile_copies(m):
        return [tile_copies(wd_hbm, wd_buf, j, down_sems.at[m], top=BAND)
                for j in range(down_edges[m], down_edges[m + 1])]

    def tick(step):
        slot = step % TICK_DEPTH
        return pltpu.make_async_copy(tick_src, tick_dst.at[slot], tick_sems.at[slot])

    wr_copy = pltpu.make_async_copy(wr_hbm, wr_buf, wr_sem)
    mid_copy = rows_copy(wd_hbm, wd_buf, BAND + PACED, lo - OVERLAP, mid_sem)
    overlap_copy = rows_copy(wd_hbm, wd_buf, lo - OVERLAP, lo, overlap_sem)
    band_copy = rows_copy(wd_hbm, wd_buf, 0, BAND, band_sem)

    sub = lax.broadcasted_iota(i32, (8, LANES), 0)
    lane = lax.broadcasted_iota(i32, (8, LANES), 1)
    state = {}

    def router(j0, j1):
        if j0 == 0:
            wr_copy.wait()
            _wait_all(x_buf, x_sem)
            state["w"] = jnp.broadcast_to(wr_buf[...].reshape(1, D), (8, D))
            state["score"] = [jnp.zeros((8, LANES), f32) for _ in range(n_blocks // 8)]
        r = jnp.dot(state["w"], x_buf[:, _tiles(j0, j1)], preferred_element_type=f32)
        for j in range(j0, j1):
            state["score"][j // 8] = jnp.where(sub == j % 8, r[:, _tiles(j - j0, j - j0 + 1)],
                                               state["score"][j // 8])

    def top_k(c0, c1):
        if c0 == 0:
            state["keys"] = []
            for q, r in enumerate(state["score"]):
                r = _round(r)
                bits = jnp.where(r == 0.0, 0, pltpu.bitcast(r, i32))
                rank = lax.shift_right_logical(jnp.where(bits < 0, ~bits, bits ^ (-2 ** 31)), 16)
                rank = jnp.where(r != r, 0, rank)
                token = (q * 8 + sub) * LANES + lane
                state["keys"].append(pltpu.bitcast(0x20000000 | (rank * S) | (S - 1 - token), f32))
            state["top"] = jnp.zeros((8, LANES), f32)
        for c in range(c0, c1):
            best = functools.reduce(jnp.maximum, state["keys"])
            best = jnp.max(jnp.max(best, axis=0, keepdims=True), axis=1, keepdims=True)
            state["top"] = jnp.where(sub == c, best, state["top"])
            state["keys"] = [jnp.where(k == best, 0.0, k) for k in state["keys"]]

    def decode():
        bits = pltpu.bitcast(state["top"], i32)
        rank = lax.shift_right_logical(bits, S.bit_length() - 1) & 0xFFFF
        score = pltpu.bitcast(jnp.where(rank >= 0x8000, rank & 0x7FFF, rank ^ 0xFFFF) << 16, f32)
        state["weight"] = _round(jax.nn.sigmoid(score))[:, :1]
        token = (S - 1) - (bits & (S - 1))
        state["token"] = [token[c, 0] for c in range(CAPACITY)]
        touched = functools.reduce(jnp.bitwise_or, [1 << (t >> 7) for t in state["token"]])
        n_early, n_late = 0, n_blocks - CAPACITY
        for j in BLOCK_ORDER:
            early = jnp.logical_and(((touched >> j) & 1) == 0, n_early < n_blocks - CAPACITY)
            order_ref[jnp.where(early, n_early, n_late)] = j
            n_early = n_early + early.astype(i32)
            n_late = n_late + 1 - early.astype(i32)

    def gather(c):
        t = state["token"][c]
        words = pltpu.bitcast(x_buf[:, pl.ds(pl.multiple_of((t >> 7) * LANES, LANES), LANES)], i32)
        lanes = lax.broadcasted_iota(i32, words.shape, 1)
        only = pltpu.bitcast(jnp.where(lanes == (t & (LANES - 1)), words, 0), bf16)
        row = lax.dot_general(jnp.ones((8, LANES), bf16), only, NT, preferred_element_type=f32)
        sel_ref[c:c + 1, :] = row[c:c + 1]

    def residual(j0, j1):
        for j in range(j0, j1):
            v = x_buf[:, _tiles(j, j + 1)].astype(f32)
            out_buf[j] = (v + v * 0.0).astype(bf16)

    def gate(j0, j1):
        if j0 == 0:
            _wait_all(wg_buf, wg_sem)
        cols = _tiles(j0, j1)
        g = _round(jnp.dot(sel_ref[...].astype(bf16), wg_buf[:, cols], preferred_element_type=f32))
        g_ref[:, cols] = _round(jax.nn.silu(g))

    def up(j0, j1):
        if j0 == 0:
            _wait_all(wu_buf, wu_sem)
        cols = _tiles(j0, j1)
        u = _round(jnp.dot(sel_ref[...].astype(bf16), wu_buf[:, cols], preferred_element_type=f32))
        h_ref[:, cols] = g_ref[:, cols] * u

    def down_tiles(m):
        for pair in wd_tile_copies(m):
            for copy in pair:
                copy.wait()
        cols = _tiles(down_edges[m], down_edges[m + 1])
        w = jnp.concatenate([wd_buf[BAND:BAND + PACED, cols], wd_buf[lo:D, cols]], axis=0)
        y = lax.dot_general(h_ref[:, cols].astype(bf16), w, NT, preferred_element_type=f32)
        y_ref[...] = y if m == 0 else y_ref[...] + y

    def down_rows(r0, r1):
        return lax.dot_general(h_ref[...].astype(bf16), wd_buf[r0:r1, :], NT, preferred_element_type=f32)

    def routed_columns(y, sel):
        update = _round(sel * 0.0 + _round(_round(y) * state["weight"]))
        rows = jnp.concatenate([sel + update, jnp.zeros((LANES - CAPACITY, y.shape[1]), f32)], axis=0)
        return pltpu.bitcast(rows.T.astype(bf16), i32)

    def write_block(slot, r0, r1, patch):
        b = order_ref[slot]
        if patch:
            token = b * LANES + lax.broadcasted_iota(i32, (1, LANES), 1)
            src = jnp.full((1, LANES), -1, i32)
            for c in range(CAPACITY):
                src = jnp.where(token == state["token"][c], c, src)
            routed = routed_ref[r0 // 2:r1 // 2, :]
            pick = jnp.broadcast_to(jnp.maximum(src, 0), routed.shape)
            new = pltpu.bitcast(jnp.take_along_axis(routed, pick, axis=1), bf16).astype(f32)
            keep = jnp.broadcast_to(src < 0, new.shape)
            out_buf[b, r0:r1, :] = jnp.where(keep, out_buf[b, r0:r1, :].astype(f32), new).astype(bf16)
        cols = pl.ds(pl.multiple_of(b * LANES, LANES), LANES)
        pltpu.make_async_copy(out_buf.at[b, r0:r1], out_hbm.at[r0:r1, cols], out_sem).start()

    def write_blocks(first, r0, r1, patch, unroll=False):
        def body(k, carry):
            write_block(first + 2 * k, r0, r1, patch)
            write_block(first + 2 * k + 1, r0, r1, patch)
            return carry

        lax.fori_loop(0, CAPACITY // 2, body, 0, unroll=unroll)

    P = functools.partial
    res_edges = (0, 3, 6, 9, 12, 14, 16)
    tasks = {}
    for first, run in (
        (ROUTER_STEP, [P(router, j, j + 2) for j in range(0, n_blocks, 2)]
         + [P(top_k, c, c + 2) for c in range(0, CAPACITY, 2)] + [decode]
         + [P(gather, c) for c in range(CAPACITY)]
         + [P(residual, a, b) for a, b in zip(res_edges, res_edges[1:])]),
        (GATE_STEP, [P(gate, j, j + 2) for j in range(0, n_tiles, 2)]),
        (UP_STEP, [P(up, j, j + 3) for j in range(0, n_tiles, 3)]
         + [P(down_tiles, m) for m in range(len(DOWN_TILES) - 1)]),
    ):
        assert all(step < first for step in tasks)
        tasks.update(enumerate(run, first))

    paced = ([tile_copies(x_hbm, x_buf, j, x_sem) for j in range(n_blocks)]
             + [tile_copies(wg_hbm, wg_buf, j, wg_sem) for j in range(n_tiles)]
             + [tile_copies(wu_hbm, wu_buf, j, wu_sem) for j in range(n_tiles)]
             + [pair for m in range(len(DOWN_TILES)) for pair in wd_tile_copies(m)])
    n_steps = len(paced) - LEAD

    rows_copy(x_hbm, x_buf, PACED, lo, x_sem).start(priority=1)
    for pair in paced[:LEAD]:
        for copy in pair:
            copy.start(priority=0)
    tick_src[...] = jnp.zeros(tick_src.shape, i32)
    for step in range(1, TICK_DEPTH + 1):
        tick(step).start()
    wr_copy.start()
    rows_copy(wg_hbm, wg_buf, PACED, lo, wg_sem).start(priority=1)
    rows_copy(wu_hbm, wu_buf, PACED, lo, wu_sem).start(priority=1)
    mid_copy.start(priority=1)
    overlap_copy.start(priority=1)
    band_copy.start(priority=1)

    for step, pair in enumerate(paced[LEAD:], 1):
        tick(step).wait()
        for copy in pair:
            copy.start(priority=0)
        if step + TICK_DEPTH <= n_steps:
            tick(step + TICK_DEPTH).start()
        if step in tasks:
            tasks.pop(step)()
    for step in sorted(tasks):
        tasks[step]()

    mid_copy.wait()
    write_blocks(0, 0, D, patch=False)

    overlap_copy.wait()
    down_tiles(len(DOWN_TILES) - 1)
    y_mid = down_rows(BAND + PACED, lo)
    sel = jnp.concatenate([sel_ref[:, BAND:BAND + PACED], sel_ref[:, lo:D]], axis=1)
    routed = routed_columns(y_ref[...], sel)
    routed_ref[BAND // 2:(BAND + PACED) // 2, :] = routed[:PACED // 2]
    routed_ref[lo // 2:, :] = routed[PACED // 2:]
    routed_ref[(BAND + PACED) // 2:lo // 2, :] = routed_columns(y_mid, sel_ref[:, BAND + PACED:lo])
    write_blocks(n_blocks - CAPACITY, BAND, D, patch=True)

    band_copy.wait()
    routed_ref[:BAND // 2, :] = routed_columns(down_rows(0, BAND), sel_ref[:, :BAND])
    write_blocks(n_blocks - CAPACITY, 0, BAND, patch=True, unroll=True)
    _wait_all(out_hbm, out_sem)


@jax.jit
def pallas_standalone__moe_arch_mod__prompt_kernel(
    x: jax.Array,
    w_r: jax.Array,
    w_gate: jax.Array,
    w_up: jax.Array,
    w_down: jax.Array,
):
    B, S, D = x.shape
    F = w_gate.shape[1]
    assert B == 1 and S == 2 * CAPACITY * LANES and F == sum(DOWN_TILES) * LANES
    assert D % 16 == 0 and D > 2 * PACED + BAND

    hbm = pl.BlockSpec(memory_space=pltpu.HBM)
    out_t = pl.pallas_call(
        _kernel,
        out_shape=jax.ShapeDtypeStruct((D, S), x.dtype),
        in_specs=[hbm] * 5,
        out_specs=hbm,
        scratch_shapes=[
            pltpu.VMEM((D, S), bf16),
            pltpu.VMEM((D,), bf16),
            pltpu.VMEM((D, F), bf16),
            pltpu.VMEM((D, F), bf16),
            pltpu.VMEM((D, F), bf16),
            pltpu.VMEM((S // LANES, D, LANES), bf16),
            pltpu.VMEM((CAPACITY, D), f32),
            pltpu.VMEM((CAPACITY, F), f32),
            pltpu.VMEM((CAPACITY, F), f32),
            pltpu.VMEM((CAPACITY, 2 * PACED), f32),
            pltpu.VMEM((D // 2, LANES), i32),
            pltpu.SMEM((S // LANES,), i32),
            pltpu.VMEM((TICK_ROWS, LANES), i32),
            pltpu.SMEM((TICK_DEPTH, TICK_ROWS, LANES), i32),
            pltpu.SemaphoreType.DMA((8,)),
            pltpu.SemaphoreType.DMA((len(DOWN_TILES),)),
            pltpu.SemaphoreType.DMA((TICK_DEPTH,)),
        ],
        compiler_params=pltpu.CompilerParams(
            vmem_limit_bytes=64 * 1024 * 1024,
            disable_semaphore_checks=True,
        ),
        name="mod_block",
    )(x.reshape(S, D).T, w_r, w_gate, w_up, w_down.T)
    return out_t.T.reshape(B, S, D)
```
